```python
import os as _os
_os.environ.setdefault("JAX_PLATFORMS", "cpu")
import jax
import jax.numpy as jnp

def _softmax(x, axis=-1):
    return jax.nn.softmax(x, axis=axis)
def _gelu(x):
    return jax.nn.gelu(x, approximate=True)
def _silu(x):
    return jax.nn.silu(x)
def _sigmoid(x):
    return jax.nn.sigmoid(x)
def _layernorm(x, axis=-1, eps=1e-5):
    m = jnp.mean(x, axis=axis, keepdims=True)
    v = jnp.var(x, axis=axis, keepdims=True)
    return (x - m) / jnp.sqrt(v + eps)
def _scatter_add(tgt, idx, src, axis=0):
    return tgt.at[idx].add(src)
def _segment_sum(src, seg, n):
    return jax.ops.segment_sum(src, seg, n)
class _Rng:
    def __init__(self, key):
        self._k = key
    def _next(self):
        self._k, sub = jax.random.split(self._k)
        return sub
    def normal(self, shape):
        return jax.random.normal(self._next(), shape, dtype=jnp.bfloat16)
    def randint(self, lo, hi, shape):
        return jax.random.randint(self._next(), shape, lo, hi, dtype=jnp.int32)
    def uniform(self, shape, lo=0.0, hi=1.0):
        return jax.random.uniform(self._next(), shape, jnp.bfloat16, lo, hi)
    def permutation(self, n):
        return jax.random.permutation(self._next(), n)


kernel_name = 'standalone__gqa_block_cached__near_ridge'

def setup_inputs():
    _rng = _Rng(jax.random.key(int.from_bytes(__import__("os").urandom(4), "little")))
    _w = (lambda a: (lambda t: t.astype(jnp.bfloat16) if jnp.issubdtype(t.dtype, jnp.floating) else t)(jnp.asarray(a)))
    B, Sq, D = 8, 96, 448
    Hq, Hkv, Sk, Dh = 16, 8, 2048, 256
    assert Hq % Hkv == 0, (Hq, Hkv)
    return {
        "x": _w((lambda *s: _rng.normal(s) * 0.8)(B, Sq, D)),
        "k_cache": _w((lambda *s: _rng.normal(s) * 0.8)(B, Hkv, Sk, Dh)),
        "v_cache": _w((lambda *s: _rng.normal(s) * 0.05)(B, Hkv, Sk, Dh)),
        "wq": _w((lambda *s: _rng.normal(s) * 0.8)(D, Hq * Dh) * (D ** -0.5)),
        "wo": _w((lambda *s: _rng.normal(s) * 0.05)(Hq * Dh, D) * ((Hq * Dh) ** -0.5)),
    }

def reference(x, k_cache, v_cache, wq, wo):
    B, Sq, D = x.shape
    Hq, Dh = 16, 256
    Hkv = k_cache.shape[1]
    rep = Hq // Hkv
    q = (lambda x, *d: x.transpose(*d))((x @ wq).reshape(B, Sq, Hq, Dh), 0, 2, 1, 3)
    k = jnp.repeat(k_cache, rep, axis=1)
    v = jnp.repeat(v_cache, rep, axis=1)
    scores = jnp.einsum("bhqd,bhkd->bhqk", q, k) * (Dh ** -0.5)
    p = _softmax(scores, axis=-1)
    o = jnp.einsum("bhqk,bhkd->bhqd", p, v)
    return (lambda x, *d: x.transpose(*d))(o, 0, 2, 1, 3).reshape(B, Sq, Hq * Dh) @ wo
```

```python
import functools
import jax
import jax.numpy as jnp
from jax import lax
from jax.experimental import pallas as pl
from jax.experimental.pallas import tpu as pltpu

LOG2E = 1.4426950408889634

def build(x, k_cache, v_cache, wq, wo, *, nslot=6, vmem=64, nc=4, exp2=False, order='qao', unroll=1, nocomp=False):
    B, Sq, D = x.shape
    _, Hkv, Sk, Dh = k_cache.shape
    Hq = wq.shape[1] // Dh
    rep = Hq // Hkv
    R = rep * Sq
    W = rep * Dh
    T = B * Hkv
    scale = Dh ** -0.5
    if exp2:
        scale = scale * LOG2E
    wot = wo.T
    k3 = k_cache.reshape(T, Sk, Dh)
    v3 = v_cache.reshape(T, Sk, Dh)
    expf = jnp.exp2 if exp2 else jnp.exp
    U = unroll
    NQ = 2 if U == 1 else 4
    npre = nslot - U

    def kernel(x_hbm, wq_hbm, wo_hbm, k_hbm, v_hbm, out_hbm,
               x_buf, wq_buf, wo_buf, kbuf, vbuf, q_buf, o_buf, acc, out_buf,
               xsem, wqsem, wosem, ksem, vsem, osem):
        def kcopy(t):
            return pltpu.make_async_copy(k_hbm.at[t], kbuf.at[t % nslot], ksem.at[t % nslot])
        def vcopy(t):
            return pltpu.make_async_copy(v_hbm.at[t], vbuf.at[t % nslot], vsem.at[t % nslot])
        def woff(h):
            return h * W if isinstance(h, int) else pl.multiple_of(h * W, W)
        def wqcopy(h):
            return pltpu.make_async_copy(wq_hbm.at[:, pl.ds(woff(h), W)], wq_buf.at[h], wqsem.at[h])
        def wocopy(h):
            return pltpu.make_async_copy(wo_hbm.at[:, pl.ds(woff(h), W)], wo_buf.at[h], wosem.at[h])
        def xcopy():
            return pltpu.make_async_copy(x_hbm, x_buf, xsem.at[0])
        def ocopy(b):
            return pltpu.make_async_copy(out_buf.at[b], out_hbm.at[b], osem.at[b])

        def when(c):
            if isinstance(c, bool):
                return (lambda f: f()) if c else (lambda f: None)
            return pl.when(c)

        def qproj(t):
            b = t // Hkv
            h = t % Hkv
            q = jnp.dot(x_buf[b], wq_buf[h], preferred_element_type=jnp.float32)
            q = (q * scale).astype(jnp.bfloat16)
            for r in range(rep):
                q_buf[t % NQ, r * Sq:(r + 1) * Sq, :] = q[:, r * Dh:(r + 1) * Dh]

        def attention(t):
            slot = t % nslot
            q = q_buf[t % NQ]
            C = Sk // nc
            ss = [lax.dot_general(q, kbuf[slot, c * C:(c + 1) * C, :], (((1,), (1,)), ((), ())), preferred_element_type=jnp.float32) for c in range(nc)]
            m = None
            for c in range(nc):
                s = ss[c]
                mc = jnp.max(s, axis=1, keepdims=True)
                if m is None:
                    mn = mc
                else:
                    mn = jnp.maximum(m, mc)
                p = expf(s - mn)
                lc = jnp.sum(p, axis=1, keepdims=True)
                oc = jnp.dot(p.astype(jnp.bfloat16), vbuf[slot, c * C:(c + 1) * C, :], preferred_element_type=jnp.float32)
                if m is None:
                    l = lc; o = oc
                else:
                    a = expf(m - mn)
                    l = l * a + lc
                    o = o * a + oc
                m = mn
            o = (o / l).astype(jnp.bfloat16)
            for r in range(rep):
                o_buf[t % NQ, :, r * Dh:(r + 1) * Dh] = o[r * Sq:(r + 1) * Sq, :]

        def oproj(t):
            if nocomp:
                acc[...] = jnp.zeros_like(acc)
                return
            h = t % Hkv
            c = lax.dot_general(o_buf[t % NQ], wo_buf[h], (((1,), (1,)), ((), ())), preferred_element_type=jnp.float32)
            if isinstance(t, int):
                if h == 0:
                    acc[...] = c
                else:
                    acc[...] += c
            else:
                acc[...] = jnp.where(h == 0, 0.0, acc[...]) + c

        def finish(t):
            b = t // Hkv
            out_buf[b] = acc[...].astype(out_buf.dtype)
            ocopy(b).start()

        def compute(t, do_q, do_o):
            if nocomp and not (isinstance(t, int) and t == 0): return
            for ch in order:
                if ch == 'q' and do_q: qproj(t + 1)
                if ch == 'a': attention(t)
                if ch == 'o' and do_o: oproj(t - 1)

        def issue(tn):
            @when(tn < T)
            def _():
                kcopy(tn).start(); vcopy(tn).start()
            @when(tn + 1 < Hkv)
            def _():
                wqcopy(tn + 1).start()
            @when(tn < Hkv)
            def _():
                wocopy(tn).start()

        def wait_w(t):
            @when(t + 1 < Hkv)
            def _():
                wqcopy(t + 1).wait()
            @when((t >= 1) & (t - 1 < Hkv))
            def _():
                wocopy(t - 1).wait()

        xcopy().start()
        wqcopy(0).start()
        def pro(t, c):
            issue(t)
            return c
        lax.fori_loop(0, npre, pro, 0)
        xcopy().wait()
        wqcopy(0).wait()
        qproj(0)

        issue(npre)
        wait_w(0)
        kcopy(0).wait(); vcopy(0).wait()
        compute(0, True, False)

        n_main = T - 2
        n_iter = n_main // U
        def body(i, carry):
            t0 = 1 + i * U
            for u in range(U):
                issue(t0 + u + npre)
            for u in range(U):
                wait_w(t0 + u)
            for u in range(U):
                kcopy(t0 + u).wait(); vcopy(t0 + u).wait()
            for u in range(U):
                compute(t0 + u, True, True)
            t = t0 + U - 1
            @pl.when((t - 1) % Hkv == Hkv - 1)
            def _():
                finish(t - 1)
            return carry
        lax.fori_loop(0, n_iter, body, 0)
        for t in range(1 + n_iter * U, T - 1):
            issue(t + npre)
            kcopy(t).wait(); vcopy(t).wait()
            compute(t, True, True)
            if (t - 1) % Hkv == Hkv - 1:
                finish(t - 1)

        t = T - 1
        kcopy(t).wait(); vcopy(t).wait()
        compute(t, False, True)
        oproj(t)
        finish(t)
        for b in range(B):
            ocopy(b).wait()

    out = pl.pallas_call(
        kernel,
        in_specs=[pl.BlockSpec(memory_space=pl.ANY)] * 5,
        out_specs=pl.BlockSpec(memory_space=pl.ANY),
        out_shape=jax.ShapeDtypeStruct((B, Sq, D), x.dtype),
        scratch_shapes=[
            pltpu.VMEM((B, Sq, D), jnp.bfloat16),
            pltpu.VMEM((Hkv, D, W), jnp.bfloat16),
            pltpu.VMEM((Hkv, D, W), jnp.bfloat16),
            pltpu.VMEM((nslot, Sk, Dh), jnp.bfloat16),
            pltpu.VMEM((nslot, Sk, Dh), jnp.bfloat16),
            pltpu.VMEM((NQ, R, Dh), jnp.bfloat16),
            pltpu.VMEM((NQ, Sq, W), jnp.bfloat16),
            pltpu.VMEM((Sq, D), jnp.float32),
            pltpu.VMEM((B, Sq, D), jnp.bfloat16),
            pltpu.SemaphoreType.DMA((1,)),
            pltpu.SemaphoreType.DMA((Hkv,)),
            pltpu.SemaphoreType.DMA((Hkv,)),
            pltpu.SemaphoreType.DMA((nslot,)),
            pltpu.SemaphoreType.DMA((nslot,)),
            pltpu.SemaphoreType.DMA((B,)),
        ],
        compiler_params=pltpu.CompilerParams(vmem_limit_bytes=vmem * 1024 * 1024),
    )(x, wq, wot, k3, v3)
    return out


@jax.jit
def pallas_standalone__gqa_block_cached__near_ridge_kernel(x, k_cache, v_cache, wq, wo):
    return build(x, k_cache, v_cache, wq, wo, nslot=4)
```

```python
import jax
import jax.numpy as jnp
from jax import lax
from jax.experimental import pallas as pl
from jax.experimental.pallas import tpu as pltpu

_NSLOT = 8
_NPRE = 6
_NCHUNK = 4
_NSUB = 2
_HROWS = 64


def _build(x, k_cache, v_cache, wq, wo):
    B, Sq, D = x.shape
    _, Hkv, Sk, Dh = k_cache.shape
    Hq = wq.shape[1] // Dh
    rep = Hq // Hkv
    R = rep * Sq
    W = rep * Dh
    T = B * Hkv
    M = B * Sq
    nslot, npre, nc, sub, hr = _NSLOT, _NPRE, _NCHUNK, _NSUB, _HROWS
    assert Hq == rep * Hkv and Hkv & (Hkv - 1) == 0 and nslot & (nslot - 1) == 0
    assert 1 < npre < nslot <= T
    LH = Hkv.bit_length() - 1
    C = Sk // nc
    CS = C // sub
    HR = nc * sub * hr
    assert C * nc == Sk and CS * sub == C and HR < Sk
    scale = Dh ** -0.5
    f32, bf16 = jnp.float32, jnp.bfloat16
    nt_dims = (((1,), (1,)), ((), ()))

    def kernel(x_hbm, wq_hbm, wo_hbm, k_hbm, v_hbm, out_hbm,
               x_buf, wq_buf, wo_buf, kbuf, vbuf, q_all, acc, out_buf,
               xsem, wqsem, wosem, ksem, vsem, osem):
        def slot_of(t):
            return t & (nslot - 1)

        def full(hbm, buf, sem, t):
            s = slot_of(t)
            return pltpu.make_async_copy(hbm.at[t], buf.at[s], sem.at[s])

        def low(hbm, buf, sem, t):
            s = slot_of(t)
            return pltpu.make_async_copy(hbm.at[t, pl.ds(HR, Sk - HR)], buf.at[s, pl.ds(HR, Sk - HR)], sem.at[s])

        def high(hbm, buf, sem, t, j):
            s = slot_of(t)
            return pltpu.make_async_copy(hbm.at[t, pl.ds(j * hr, hr)], buf.at[s, pl.ds(j * hr, hr)], sem.at[s])

        def woff(h):
            return h * W if isinstance(h, int) else pl.multiple_of(h * W, W)

        def wqcopy(h):
            return pltpu.make_async_copy(wq_hbm.at[:, pl.ds(woff(h), W)], wq_buf.at[h], wqsem.at[h])

        def wocopy(h):
            return pltpu.make_async_copy(wo_hbm.at[:, pl.ds(woff(h), W)], wo_buf.at[h], wosem.at[h])

        def xcopy():
            return pltpu.make_async_copy(x_hbm, x_buf, xsem.at[0])

        def ocopy(b):
            return pltpu.make_async_copy(out_buf.at[b], out_hbm.at[b], osem.at[b])

        def issue_low(tn):
            low(k_hbm, kbuf, ksem, tn).start(priority=1)
            low(v_hbm, vbuf, vsem, tn).start(priority=1)

        def oproj(t, o):
            h = t & (Hkv - 1)
            c = lax.dot_general(o, wo_buf[h], nt_dims, preferred_element_type=f32)
            if isinstance(t, int):
                if h == 0:
                    acc[...] = c
                else:
                    acc[...] += c
            else:
                acc[...] = jnp.where(h == 0, 0.0, acc[...]) + c

        def finish(t):
            b = t >> LH
            out_buf[b] = acc[...].astype(out_buf.dtype)
            ocopy(b).start()

        def step(t, o_prev, last=False):
            slot = slot_of(t)
            full(k_hbm, kbuf, ksem, t).wait()
            q = q_all[t]
            ss = []
            for c in range(nc):
                parts = []
                for u in range(sub):
                    r0 = c * C + u * CS
                    parts.append(lax.dot_general(q, kbuf[slot, r0:r0 + CS, :], nt_dims, preferred_element_type=f32))
                    if not last:
                        high(k_hbm, kbuf, ksem, t + 1, c * sub + u).start()
                ss.append(jnp.concatenate(parts, axis=1))
            if o_prev is not None:
                oproj(t - 1, o_prev)
            m = None
            stats = []
            for c in range(nc):
                s = ss[c]
                mc = jnp.max(s, axis=1, keepdims=True)
                mn = mc if m is None else jnp.maximum(m, mc)
                p = jnp.exp(s - mn)
                lc = jnp.sum(p, axis=1, keepdims=True)
                a = None if m is None else jnp.exp(m - mn)
                stats.append((p.astype(bf16), lc, a))
                m = mn
            full(v_hbm, vbuf, vsem, t).wait()
            o = l = None
            for c in range(nc):
                pb, lc, a = stats[c]
                oc = None
                for u in range(sub):
                    r0 = c * C + u * CS
                    d = jnp.dot(pb[:, u * CS:(u + 1) * CS], vbuf[slot, r0:r0 + CS, :], preferred_element_type=f32)
                    oc = d if oc is None else oc + d
                    if not last:
                        high(v_hbm, vbuf, vsem, t + 1, c * sub + u).start()
                if a is None:
                    l, o = lc, oc
                else:
                    l = l * a + lc
                    o = o * a + oc
            o = (o / l).astype(bf16)
            return jnp.concatenate([o[r * Sq:(r + 1) * Sq, :] for r in range(rep)], axis=1)

        xcopy().start(priority=1)

        def start_wq(h, c):
            wqcopy(h).start(priority=1)
            return c
        lax.fori_loop(0, Hkv, start_wq, 0)

        def start_wo(h, c):
            wocopy(h).start(priority=1)
            return c
        lax.fori_loop(0, Hkv, start_wo, 0)

        def start_first(t, c):
            full(k_hbm, kbuf, ksem, t).start(priority=1)
            full(v_hbm, vbuf, vsem, t).start(priority=1)
            return c
        lax.fori_loop(0, 1, start_first, 0)

        def start_kv(t, c):
            issue_low(t)
            return c
        lax.fori_loop(1, npre, start_kv, 0)

        xcopy().wait()

        def qbody(h, c):
            wqcopy(h).wait()
            q = jnp.dot(x_buf[...], wq_buf[h], preferred_element_type=f32)
            q = (q * scale).astype(bf16)
            for b in range(B):
                for r in range(rep):
                    q_all[b * Hkv + h, r * Sq:(r + 1) * Sq, :] = q[b * Sq:(b + 1) * Sq, r * Dh:(r + 1) * Dh]
            return c
        lax.fori_loop(0, Hkv, qbody, 0)
        for h in range(Hkv):
            wocopy(h).wait()

        issue_low(npre)
        o = step(0, None)

        def body(t, o):
            @pl.when(t + npre < T)
            def _():
                issue_low(t + npre)
            o = step(t, o)

            @pl.when(((t - 1) & (Hkv - 1)) == Hkv - 1)
            def _():
                finish(t - 1)
            return o
        o = lax.fori_loop(1, T - 1, body, o)

        o = step(T - 1, o, last=True)
        oproj(T - 1, o)
        finish(T - 1)
        for b in range(B):
            ocopy(b).wait()

    return pl.pallas_call(
        kernel,
        in_specs=[pl.BlockSpec(memory_space=pl.ANY)] * 5,
        out_specs=pl.BlockSpec(memory_space=pl.ANY),
        out_shape=jax.ShapeDtypeStruct((B, Sq, D), x.dtype),
        scratch_shapes=[
            pltpu.VMEM((M, D), bf16),
            pltpu.VMEM((Hkv, D, W), bf16),
            pltpu.VMEM((Hkv, D, W), bf16),
            pltpu.VMEM((nslot, Sk, Dh), bf16),
            pltpu.VMEM((nslot, Sk, Dh), bf16),
            pltpu.VMEM((T, R, Dh), bf16),
            pltpu.VMEM((Sq, D), f32),
            pltpu.VMEM((B, Sq, D), bf16),
            pltpu.SemaphoreType.DMA((1,)),
            pltpu.SemaphoreType.DMA((Hkv,)),
            pltpu.SemaphoreType.DMA((Hkv,)),
            pltpu.SemaphoreType.DMA((nslot,)),
            pltpu.SemaphoreType.DMA((nslot,)),
            pltpu.SemaphoreType.DMA((B,)),
        ],
        compiler_params=pltpu.CompilerParams(
            vmem_limit_bytes=64 * 1024 * 1024,
            disable_bounds_checks=True,
        ),
    )(x.reshape(M, D), wq, wo.T, k_cache.reshape(T, Sk, Dh), v_cache.reshape(T, Sk, Dh))


@jax.jit
def pallas_standalone__gqa_block_cached__near_ridge_kernel(
    x: jax.Array,
    k_cache: jax.Array,
    v_cache: jax.Array,
    wq: jax.Array,
    wo: jax.Array,
):
    return _build(x, k_cache, v_cache, wq, wo)
```
